```python
import os as _os
_os.environ.setdefault("JAX_PLATFORMS", "cpu")
import jax
import jax.numpy as jnp

def _softmax(x, axis=-1):
    return jax.nn.softmax(x, axis=axis)
def _gelu(x):
    return jax.nn.gelu(x, approximate=True)
def _silu(x):
    return jax.nn.silu(x)
def _sigmoid(x):
    return jax.nn.sigmoid(x)
def _layernorm(x, axis=-1, eps=1e-5):
    m = jnp.mean(x, axis=axis, keepdims=True)
    v = jnp.var(x, axis=axis, keepdims=True)
    return (x - m) / jnp.sqrt(v + eps)
def _scatter_add(tgt, idx, src, axis=0):
    return tgt.at[idx].add(src)
def _segment_sum(src, seg, n):
    return jax.ops.segment_sum(src, seg, n)
class _Rng:
    def __init__(self, key):
        self._k = key
    def _next(self):
        self._k, sub = jax.random.split(self._k)
        return sub
    def normal(self, shape):
        return jax.random.normal(self._next(), shape, dtype=jnp.bfloat16)
    def randint(self, lo, hi, shape):
        return jax.random.randint(self._next(), shape, lo, hi, dtype=jnp.int32)
    def uniform(self, shape, lo=0.0, hi=1.0):
        return jax.random.uniform(self._next(), shape, jnp.bfloat16, lo, hi)
    def permutation(self, n):
        return jax.random.permutation(self._next(), n)


kernel_name = 'concat_heads__linear_kernel_hedgehog__ssm_conv_s5__prompt'

def setup_inputs():
    _rng = _Rng(jax.random.key(int.from_bytes(__import__("os").urandom(4), "little")))
    _w = (lambda a: (lambda t: t.astype(jnp.bfloat16) if jnp.issubdtype(t.dtype, jnp.floating) else t)(jnp.asarray(a)))
    def _A_setup():
        B, S, D, H = 1, 2048, 640, 32
        Dh = D // H
        return {
            "x": _w((lambda *s: _rng.normal(s) * 0.4)(B, S, D)),
            "wqkv": _w((lambda *s: _rng.normal(s) * 0.4)(D, 3 * D)),
            "w_phi": _w((lambda *s: _rng.normal(s) * 0.4)(H, Dh, Dh) * (Dh ** -0.5)),
            "wo": _w((lambda *s: _rng.normal(s) * 0.05)(D, D)),
        }
    _A_in = _A_setup()

    def _B_setup():
        B, S, D = 1, 2048, 640
        P = D
        Lambda_re = -0.5 * jnp.exp((lambda *s: _rng.normal(s) * 0.8)(P))
        Lambda_im = (lambda *s: _rng.normal(s) * 0.8)(P) * 1.0
        B_re = (lambda *s: _rng.normal(s) * 0.8)(P, D) * (D ** -0.5)
        B_im = (lambda *s: _rng.normal(s) * 0.8)(P, D) * (D ** -0.5)
        C_re = (lambda *s: _rng.normal(s) * 0.8)(D, P) * (P ** -0.5)
        C_im = (lambda *s: _rng.normal(s) * 0.8)(D, P) * (P ** -0.5)
        log_dt = (lambda *s: _rng.normal(s) * 0.8)(P) * 0.3 - 2.0
        Dskip = (lambda *s: _rng.normal(s) * 0.8)(D)
        return {
            "x": _w((lambda *s: _rng.normal(s) * 0.05)(B, S, D)),
            "Lambda_re": _w(Lambda_re),
            "Lambda_im": _w(Lambda_im),
            "B_re": _w(B_re),
            "B_im": _w(B_im),
            "C_re": _w(C_re),
            "C_im": _w(C_im),
            "log_dt": _w(log_dt),
            "Dskip": _w(Dskip),
        }
    _B_in = _B_setup()

    return {
        "A_x": _A_in["x"],
        "A_wqkv": _A_in["wqkv"],
        "A_w_phi": _A_in["w_phi"],
        "A_wo": _A_in["wo"],
        "B_x": _B_in["x"],
        "B_Lambda_re": _B_in["Lambda_re"],
        "B_Lambda_im": _B_in["Lambda_im"],
        "B_B_re": _B_in["B_re"],
        "B_B_im": _B_in["B_im"],
        "B_C_re": _B_in["C_re"],
        "B_C_im": _B_in["C_im"],
        "B_log_dt": _B_in["log_dt"],
        "B_Dskip": _B_in["Dskip"],
    }

def reference(A_x, A_wqkv, A_w_phi, A_wo, B_x, B_Lambda_re, B_Lambda_im, B_B_re, B_B_im, B_C_re, B_C_im, B_log_dt, B_Dskip):
    def _A_ref(x, wqkv, w_phi, wo):
        B, S, D = x.shape
        H = 32; Dh = D // H
        qkv = (lambda x, *d: x.transpose(*d))((x @ wqkv).reshape(B, S, 3, H, Dh), 2, 0, 3, 1, 4)
        q, k, v = qkv[0], qkv[1], qkv[2]
        pq = jnp.einsum("bhsd,hdf->bhsf", q, w_phi)
        pk = jnp.einsum("bhsd,hdf->bhsf", k, w_phi)
        phi_q = jnp.concatenate([_softmax(pq, axis=-1), _softmax(-pq, axis=-1)], axis=-1)
        phi_k = jnp.concatenate([_softmax(pk, axis=-1), _softmax(-pk, axis=-1)], axis=-1)
        kv = jnp.einsum("bhsf,bhsd->bhfd", phi_k, v)
        z  = jnp.einsum("bhsf->bhf", phi_k)
        num = jnp.einsum("bhqf,bhfd->bhqd", phi_q, kv)
        den = jnp.einsum("bhqf,bhf->bhq", phi_q, z)[..., None] + 1e-6
        o = num / den
        return (lambda x, *d: x.transpose(*d))(o, 0, 2, 1, 3).reshape(B, S, D) @ wo

    def _B_ref(x, Lambda_re, Lambda_im, B_re, B_im, C_re, C_im, log_dt, Dskip):
        Bsz, L, H = x.shape
        Lam = Lambda_re + 1j * Lambda_im
        Bmat = B_re + 1j * B_im
        Cmat = C_re + 1j * C_im
        dt = jnp.exp(log_dt)
        Lam_bar = jnp.exp(dt * Lam)
        B_bar = ((Lam_bar - 1.0) / Lam)[:, None] * Bmat
        Bu = jnp.einsum("bld,pd->blp", x + 0j, B_bar)
        h = jnp.zeros_like(Bu[:, 0, :])
        hs = []
        for t in range(L):
            h = Lam_bar[None, :] * h + Bu[:, t, :]
            hs.append(h)
        hseq = jnp.stack(hs, 1)
        y = 2.0 * jnp.einsum("blp,dp->bld", hseq, Cmat).real + x * Dskip[None, None, :]
        return y

    a = _A_ref(A_x, A_wqkv, A_w_phi, A_wo)
    b = _B_ref(B_x, B_Lambda_re, B_Lambda_im, B_B_re, B_B_im, B_C_re, B_C_im, B_log_dt, B_Dskip)
    return jnp.concatenate([a, b], axis=-1)
```

```python
import math

import jax
import jax.numpy as jnp
import jax.experimental.pallas as pl
import jax.experimental.pallas.tpu as pltpu

UA, UC = 2, 2
SA, SY, SO, SB = 0, 0, 0, 0
MH = 320
CP = 1
FP = 0

S = 2048
D = 640
H = 32
DH = 20
TB = 256
NB = S // TB
NCH = 8
C = TB // NCH
WS = C // 2 + 4
NL = D // 128
NPAIR = H // 2
HB = NB // 2
NG = D // (2 * MH)
PG = NPAIR // NG
LOG2E = 1.4426950408889634

f32 = jnp.float32
bf16 = jnp.bfloat16
u32 = jnp.uint32

NN = (((1,), (0,)), ((), ()))
NT = (((1,), (1,)), ((), ()))
TN = (((0,), (0,)), ((), ()))


def _dot(a, b, dims):
    return jax.lax.dot_general(a, b, dims, preferred_element_type=f32)


def _w(x):
    return pltpu.bitcast(x.astype(bf16), u32)


def _b(x):
    return pltpu.bitcast(x, bf16)


def _cmul(ar, ai, br, bi):
    return ar * br - ai * bi, ar * bi + ai * br


def _par_red(op, rows):
    m = rows[0]
    for r in rows[1:]:
        m = op(m, r)
    m = op(m, pltpu.roll(m, 4, 0))
    m = op(m, pltpu.roll(m, 2, 0))
    return m


def _recip(x):
    r = pl.reciprocal(x, approx=True)
    return r * (2.0 - x * r)


def _phi_pair(p):
    rows = [p[8 * i:8 * i + 8] for i in range(5)]
    mx = _par_red(jnp.maximum, rows)
    mn = _par_red(jnp.minimum, rows)
    ep = [jnp.exp2(r - mx) for r in rows]
    en = [jnp.exp2(mn - r) for r in rows]
    rp = _recip(_par_red(jnp.add, ep))
    rn = _recip(_par_red(jnp.add, en))
    out = [e * rp for e in ep] + [e * rn for e in en]
    return jnp.concatenate(out, axis=0).astype(bf16)


def _s_ops(a11, a12, a21, a22):
    s1 = a21 + a22
    s2 = s1 - a11
    return a11, a12, a12 - s2, a22, s1, s2, a11 - a21


def _t_ops(b11, b12, b21, b22):
    t1 = b12 - b11
    t2 = b22 - t1
    return b11, b21, b22, t2 - b21, t1, t2, b22 - b12


def _winograd(p):
    u2 = p[0] + p[5]
    u3 = u2 + p[6]
    return p[0] + p[1], u2 + p[4] + p[2], u3 - p[3], u3 + p[4]


PORD = (0, 1, 5, 6, 4, 3, 2)


def _kernel(xa_h, wqkv_h, wphi_h, wo_h, xb_h, lre_h, lim_h, bre_h, bim_h, cre_h, cim_h, ldt_h, dsk_h,
            out_h,
            xa_v, wqkv_v, wphi_v, wo_v, xb_v, lre_v, lim_v, bre_v, bim_v, cre_v, cim_v, ldt_v, dsk_v,
            out_v,
            wp_ref, wt_ref, ws_ref, wk_ref, xt_ref, phiq_ref, kv_ref, kvl_ref, c2_ref, ct_ref, wo_ref,
            tab_ref, carry_ref, zero_ref, xs_ref, bu_ref, hs_ref, fg_ref,
            sem_in, sem_out):

    def cp(src, dst, k):
        return pltpu.make_async_copy(src, dst, sem_in.at[k])

    def xb_cp(lo, hi, k):
        r = pl.ds(TB * lo, TB * (hi - lo))
        return cp(xb_h.at[r], xb_v.at[r], k)

    g0 = [cp(lre_h, lre_v, 0), cp(lim_h, lim_v, 1), cp(ldt_h, ldt_v, 2), cp(wphi_h, wphi_v, 7)]
    g1 = [cp(bre_h, bre_v, 3), xb_cp(0, 1, 4), cp(bim_h, bim_v, 5)]
    g1b = [xb_cp(1, HB, 14)]
    g2 = [xb_cp(HB, NB, 6), cp(wqkv_h, wqkv_v, 10)]
    g3 = [cp(xa_h, xa_v, 12), cp(wo_h, wo_v, 13), cp(dsk_h, dsk_v, 11)]
    gc = [cp(cre_h, cre_v, 8), cp(cim_h, cim_v, 9)]
    if CP == 0:
        g2 = g2 + gc
    else:
        g3 = g3 + gc

    def out_cp(i, part):
        r = pl.ds(pl.multiple_of(TB * i, TB), TB)
        c = pl.ds(D * part, D)
        return pltpu.make_async_copy(out_v.at[r, c], out_h.at[r, c], sem_out.at[2 * i + part])

    def lam_prep():
        lre = lre_v[...].astype(f32).reshape(1, D)
        lim = lim_v[...].astype(f32).reshape(1, D)
        dt = jnp.exp(ldt_v[...].astype(f32).reshape(1, D)).astype(bf16).astype(f32)
        mag = jnp.exp(dt * lre)
        ar = mag * jnp.cos(dt * lim)
        ai = mag * jnp.sin(dt * lim)
        nr, ni = ar - 1.0, ai
        den = lre * lre + lim * lim
        tab_ref[10] = jnp.broadcast_to(2.0 * (nr * lre + ni * lim) / den, (8, D))
        tab_ref[11] = jnp.broadcast_to(2.0 * (ni * lre - nr * lim) / den, (8, D))
        ar8 = jnp.broadcast_to(ar, (8, D))
        ai8 = jnp.broadcast_to(ai, (8, D))
        tab_ref[0] = ar8
        tab_ref[1] = ai8
        pr, pi = ar8, ai8
        for _ in range(int(math.log2(C))):
            pr, pi = _cmul(pr, pi, pr, pi)
        sub = jax.lax.broadcasted_iota(jnp.int32, (8, D), 0)
        tr, ti = pr, pi
        for n, k in enumerate((1, 2, 4)):
            tab_ref[2 + 2 * n] = pr
            tab_ref[3 + 2 * n] = pi
            sr, si = pltpu.roll(tr, k, 0), pltpu.roll(ti, k, 0)
            mr, mi = _cmul(tr, ti, sr, si)
            tr = jnp.where(sub >= k, mr, tr)
            ti = jnp.where(sub >= k, mi, ti)
            pr, pi = _cmul(pr, pi, pr, pi)
        tab_ref[8] = tr
        tab_ref[9] = ti
        carry_ref[...] = jnp.zeros(carry_ref.shape, f32)
        zz = ar8[:, 0:128]
        zero_ref[...] = pltpu.bitcast(zz - zz, u32)

    def c_rows(rows, tok=None):
        cr2, ci2 = tab_ref[10], tab_ref[11]
        if tok is not None:
            tok = jnp.concatenate([tok] * NL, axis=1)
            cr2 = pltpu.bitcast(pltpu.bitcast(cr2, u32) | tok, f32)
            ci2 = pltpu.bitcast(pltpu.bitcast(ci2, u32) | tok, f32)
        cr2 = jnp.concatenate([cr2] * 2, axis=0)
        ci2 = jnp.concatenate([ci2] * 2, axis=0)
        a = cre_v[rows, :].astype(f32)
        b = cim_v[rows, :].astype(f32)
        return a * cr2 - b * ci2, -(a * ci2 + b * cr2)

    def c_prep(lo, n, tok=None):
        for r in range(n):
            if not SY:
                cr, ci = c_rows(pl.ds(pl.multiple_of(16 * (lo + r), 16), 16), tok)
                wr = pl.ds(pl.multiple_of(8 * (lo + r), 8), 8)
                c2_ref[wr, 0:D] = _w(cr)
                c2_ref[wr, D:2 * D] = _w(ci)

    def c_prep_s(r, tok=None):
        b11, b21 = c_rows(pl.ds(pl.multiple_of(16 * r, 16), 16), tok)
        b12, b22 = c_rows(pl.ds(pl.multiple_of(256 + 16 * r, 16), 16), tok)
        for n, t in enumerate(_t_ops(b11, b12, b21, b22)):
            ct_ref[n, pl.ds(pl.multiple_of(8 * r, 8), 8), :] = _w(t)

    def c_prep_tail(r, tok=None):
        cr, ci = c_rows(pl.ds(pl.multiple_of(512 + 16 * r, 16), 16), tok)
        wr = pl.ds(pl.multiple_of(8 * r, 8), 8)
        c2_ref[wr, 0:D] = _w(cr)
        c2_ref[wr, D:2 * D] = _w(ci)

    def wp_prep():
        for d in range(DH):
            t = wphi_v[d].astype(f32).T
            wp_ref[pl.ds(d, H, stride=DH), :] = jnp.concatenate(
                [t, jnp.zeros((H, 128 - DH), f32)], axis=1)

    BANDS = ((0, 160), (112, 288), (240, 400), (352, 528), (480, 640))

    def fold_lhs():
        sub = jax.lax.broadcasted_iota(jnp.int32, (8, 128), 0)
        lane = jax.lax.broadcasted_iota(jnp.int32, (8, 128), 1)
        selv = [(4 * v + (sub >> 1) == lane).astype(f32) for v in range(5)]
        off = 0
        for j, (lo, hi) in enumerate(BANDS):
            vs = range(lo // 8, hi // 8)
            sel = jnp.concatenate([selv[v % 5] for v in vs], axis=0).astype(bf16)
            full = _dot(sel, wp_ref[128 * j:128 * (j + 1), :].astype(bf16), NT)
            key = (128 * j + lane) // DH - (sub & 1)
            fg = jnp.concatenate(
                [jnp.where(key == 2 * (v // 5), full[8 * k:8 * k + 8], 0.0) for k, v in enumerate(vs)], axis=0)
            fg_ref[off:off + (hi - lo) // 2, :] = _w(fg)
            off += (hi - lo) // 2

    def fg_get(j):
        off = sum((hi - lo) // 2 for lo, hi in BANDS[:j])
        return _b(fg_ref[off:off + (BANDS[j][1] - BANDS[j][0]) // 2, :])

    def store_w(part, col):
        if not SA:
            for nt in range(NL):
                wt_ref[part * D // 2:(part + 1) * D // 2, 128 * nt:128 * (nt + 1)] = _w(col(nt))
            return
        for nt in range(2):
            lo, hi = col(nt), col(nt + 2)
            for g in range(NG):
                r0, r1, r2 = 2 * MH * g, 2 * MH * g + MH, 2 * MH * (g + 1)
                for n, m in enumerate(_s_ops(lo[r0:r1], hi[r0:r1], lo[r1:r2], hi[r1:r2])):
                    ws_ref[NG * part + g, n, :, 128 * nt:128 * (nt + 1)] = _w(m)
        w4 = col(4)
        for g in range(NG):
            wk_ref[NG * part + g] = _w(w4[2 * MH * g:2 * MH * (g + 1)])

    def fold(part):
        def col(nt):
            ps = [_dot(fg_get(j), wqkv_v[128 * nt:128 * (nt + 1), part * D + 128 * j: part * D + 128 * (j + 1)],
                       NT) * LOG2E for j in range(5)]
            return jnp.concatenate(
                [ps[0][0:112], ps[0][112:160] + ps[1][0:48], ps[1][48:128], ps[1][128:176] + ps[2][0:48],
                 ps[2][48:112], ps[2][112:160] + ps[3][0:48], ps[3][48:128], ps[3][128:176] + ps[4][0:48],
                 ps[4][48:160]], axis=0)
        store_w(part, col)

    def wv_t():
        store_w(2, lambda nt: wqkv_v[128 * nt:128 * (nt + 1), 2 * D:3 * D].T.astype(f32))
        kv_ref[...] = jnp.zeros(kv_ref.shape, f32)

    def bu_mm(i, dep=None):
        for l in range(NL):
            for j in range(NCH):
                w = pltpu.bitcast(xb_v[TB * i + C * j:TB * i + C * (j + 1), 128 * l:128 * (l + 1)], u32)
                xs_ref[i, l, pl.ds(WS * j, C // 2), :] = w
        cols = []
        for l in range(NL):
            rows = []
            for c in range(C // 2):
                v = xs_ref[i, l, pl.ds(c, 8, stride=WS), :]
                u0 = pltpu.unpack_elementwise(v, index=0, packed_dtype=bf16, unpacked_dtype=f32)
                u1 = pltpu.unpack_elementwise(v, index=1, packed_dtype=bf16, unpacked_dtype=f32)
                rows.append(jnp.concatenate([u0, u1], axis=0).astype(bf16))
            cols.append(jnp.concatenate(rows, axis=0))
        z = jnp.concatenate(cols, axis=1)
        bur = _dot(z, bre_v[...], NT)
        if dep is not None:
            z0 = _b(pltpu.bitcast(z[0:16, 0:128], u32) | dep)
            z = jnp.concatenate(
                [jnp.concatenate([z0, z[0:16, 128:]], axis=1), z[16:]], axis=0)
        return bur, _dot(z, bim_v[...], NT)

    def scan(i, bur, bui):
        ar, ai = tab_ref[0], tab_ref[1]
        hr, hi = bur[0:8], bui[0:8]
        for c in range(1, C):
            mr, mi = _cmul(ar, ai, hr, hi)
            hr, hi = mr + bur[8 * c:8 * c + 8], mi + bui[8 * c:8 * c + 8]
        sub = jax.lax.broadcasted_iota(jnp.int32, (8, D), 0)
        for n, k in enumerate((1, 2, 4)):
            sr = jnp.where(sub >= k, pltpu.roll(hr, k, 0), 0.0)
            si = jnp.where(sub >= k, pltpu.roll(hi, k, 0), 0.0)
            mr, mi = _cmul(tab_ref[2 + 2 * n], tab_ref[3 + 2 * n], sr, si)
            hr, hi = hr + mr, hi + mi
        cr, ci = carry_ref[0], carry_ref[1]
        mr, mi = _cmul(tab_ref[8], tab_ref[9], cr, ci)
        gr, gi = hr + mr, hi + mi
        carry_ref[0] = jnp.broadcast_to(gr[7:8], (8, D))
        carry_ref[1] = jnp.broadcast_to(gi[7:8], (8, D))
        hr = jnp.where(sub == 0, cr, pltpu.roll(gr, 1, 0))
        hi = jnp.where(sub == 0, ci, pltpu.roll(gi, 1, 0))
        for c in range(0, C, 2):
            mr, mi = _cmul(ar, ai, hr, hi)
            h0r, h0i = mr + bur[8 * c:8 * c + 8], mi + bui[8 * c:8 * c + 8]
            mr, mi = _cmul(ar, ai, h0r, h0i)
            hr, hi = mr + bur[8 * c + 8:8 * c + 16], mi + bui[8 * c + 8:8 * c + 16]
            pr = pltpu.pack_elementwise([h0r, hr], packed_dtype=bf16)
            pi = pltpu.pack_elementwise([h0i, hi], packed_dtype=bf16)
            for l in range(NL):
                hs_ref[i, l, pl.ds(c // 2, 8, stride=WS), :] = pr[:, 128 * l:128 * (l + 1)]
                hs_ref[i, NL + l, pl.ds(c // 2, 8, stride=WS), :] = pi[:, 128 * l:128 * (l + 1)]
        tok = pr[:, 0:128]
        for l in range(1, NL):
            tok = tok | pr[:, 128 * l:128 * (l + 1)]
        return tok & zero_ref[...]

    def y_mm(i):
        def hpart(m, k):
            return jnp.concatenate(
                [_b(jnp.concatenate([hs_ref[i, NL * k + l, pl.ds(WS * j, C // 2), :]
                                     for j in range(4 * m, 4 * m + 4)], axis=0))
                 for l in range(NL)], axis=1)
        a = [[hpart(m, k) for k in range(2)] for m in range(2)]
        rows = pl.ds(pl.multiple_of(TB * i, TB), TB)
        skip = (xb_v[rows, :] * dsk_v[...].reshape(1, D)).astype(f32)
        if not SY:
            hcat = jnp.concatenate([jnp.concatenate(a[m], axis=1) for m in range(2)], axis=0)
            y = _dot(hcat, _b(c2_ref[...]), NT)
        else:
            sa = _s_ops(a[0][0].astype(f32), a[0][1].astype(f32), a[1][0].astype(f32), a[1][1].astype(f32))
            sa = (a[0][0], a[0][1], sa[2].astype(bf16), a[1][1], sa[4].astype(bf16), sa[5].astype(bf16),
                  sa[6].astype(bf16))
            p = [None] * 7
            for n in PORD:
                p[n] = _dot(sa[n], _b(ct_ref[n]), NT)
            hcat = jnp.concatenate([jnp.concatenate(a[m], axis=1) for m in range(2)], axis=0)
            e = _dot(hcat, _b(c2_ref[0:64, :]), NT)
            c11, c12, c21, c22 = _winograd(p)
            y = jnp.concatenate([jnp.concatenate([c11, c12, e[0:128]], axis=1),
                                 jnp.concatenate([c21, c22, e[128:]], axis=1)], axis=0)
        out_v[rows, D:2 * D] = y + skip
        out_cp(i, 1).start()

    def a1(i):
        r0 = pl.multiple_of(TB * i, TB)
        if SA:
            x = [[xa_v[pl.ds(r0 + 128 * n, 128), 256 * k:256 * (k + 1)] for n in range(2)] for k in range(2)]
            t = _t_ops(x[0][0].astype(f32), x[0][1].astype(f32), x[1][0].astype(f32), x[1][1].astype(f32))
            x4 = jnp.concatenate([xa_v[pl.ds(r0 + 128 * n, 128), 512:640] for n in range(2)], axis=1)
            for n, m in enumerate((x[0][0], x[1][0], x[1][1]) + t[3:] + (x4,)):
                xt_ref[n] = _w(m)

            def proj(part, g):
                u = NG * part + g
                p = [None] * 7
                for n in PORD:
                    p[n] = _dot(_b(ws_ref[u, n]), _b(xt_ref[n]), NT)
                e = [[_dot(_b(wk_ref[u, MH // 2 * m:MH // 2 * (m + 1), :]),
                           _b(xt_ref[7, :, 128 * n:128 * n + 128]), NT) for n in range(2)] for m in range(2)]
                c11, c12, c21, c22 = _winograd(p)
                return jnp.concatenate([jnp.concatenate([c11 + e[0][0], c12 + e[0][1]], axis=1),
                                        jnp.concatenate([c21 + e[1][0], c22 + e[1][1]], axis=1)], axis=0)
            ng, pg = NG, PG
        else:
            xa = xa_v[pl.ds(r0, TB), :]

            def proj(part, g):
                return _dot(_b(wt_ref[part * D // 2 + 80 * g:part * D // 2 + 80 * (g + 1), :]), xa, NT)
            ng, pg = 4, 4

        ones = jnp.ones((8, TB), f32)
        for g in range(ng):
            if SA:
                pk = proj(1, g)
                vt = proj(2, g)
            else:
                vt = proj(2, g)
                pk = proj(1, g)
            if CP == 1:
                tok = pltpu.bitcast(vt[0:8, 0:128], u32) & zero_ref[...]
                if SY:
                    if g < 2:
                        c_prep_s(2 * i + g, tok)
                    elif g == 2:
                        c_prep_tail(i, tok)
                elif g < 3:
                    c_prep(5 * i + 2 * g, 2 if g < 2 else 1, tok)
            pq = proj(0, g)
            for q in range(pg):
                phik = _phi_pair(pk[40 * q:40 * q + 40])
                lhs = jnp.concatenate([vt[40 * q:40 * q + 40], ones], axis=0).astype(bf16)
                kv_ref[pg * g + q] += _dot(lhs, phik, NT)
            for q in range(pg):
                p = pg * g + q
                phiq_ref[i, 40 * p:40 * p + 40, :] = _w(_phi_pair(pq[40 * q:40 * q + 40]))

    def kv_final():
        m = jax.lax.broadcasted_iota(jnp.int32, (48, 80), 0)
        n = jax.lax.broadcasted_iota(jnp.int32, (48, 80), 1)
        e_row = jnp.where(m < 40, m // 20, (m - 40) // 4)
        msk = e_row == n % 2
        for p in range(NPAIR):
            kvl_ref[p] = jnp.where(msk, kv_ref[p], 0.0).astype(bf16)
        wo_ref[...] = _w(wo_v[...])

    def a2_num(i):
        sub = jax.lax.broadcasted_iota(jnp.int32, (8, TB), 0)
        parts = []
        for p in range(NPAIR):
            res = _dot(kvl_ref[p], _b(phiq_ref[i, 40 * p:40 * p + 40, :]), NN)
            r = _recip(res[40:48] + 1e-6)
            rr = pltpu.roll(r, 4, 0)
            ra = jnp.where(sub < 4, r, rr)
            rc = jnp.where(sub >= 4, r, rr)
            parts += [res[0:8] * ra, res[8:16] * ra, res[16:24] * r,
                      res[24:32] * rc, res[32:40] * rc]
        return jnp.concatenate(parts, axis=0).astype(bf16)

    def a2_out(i, ot):
        out_v[pl.ds(pl.multiple_of(TB * i, TB), TB), 0:D] = _dot(ot, _b(wo_ref[...]), TN)
        out_cp(i, 0).start()

    def loop(lo, hi, u, fn):
        def body(k, _):
            for j in range(u):
                fn(lo + k * u + j)
            return 0
        jax.lax.fori_loop(0, (hi - lo) // u, body, 0)

    def ya_block(i):
        ot = a2_num(i)
        y_mm(i)
        a2_out(i, ot)

    for c in g0 + g1:
        c.start()
    for c in g0:
        c.wait()
    lam_prep()
    wp_prep()
    fold_lhs()
    for c in g1:
        c.wait()
    for c in g1b:
        c.start()
    bur, bui = bu_mm(0)
    bu_ref[0] = bur
    bu_ref[1] = bui
    for c in g1b:
        c.wait()
    for c in g2:
        c.start()
    t0 = scan(0, bu_ref[0], bu_ref[1])
    bur, bui = bu_mm(1, t0)
    scan(1, bur, bui)
    bur, bui = bu_mm(2)
    scan(2, bur, bui)
    bur, bui = bu_mm(3)
    bu_ref[0] = bur
    bu_ref[1] = bui
    for c in g2:
        c.wait()
    for c in g3:
        c.start()
    t3 = scan(3, bu_ref[0], bu_ref[1])
    bur, bui = bu_mm(4, t3)
    scan(4, bur, bui)
    bur, bui = bu_mm(5)
    scan(5, bur, bui)
    bur, bui = bu_mm(6)
    if FP == 0:
        fold(0)
    scan(6, bur, bui)
    bur, bui = bu_mm(7)
    if FP == 1:
        fold(0)
    fold(1)
    if CP == 0:
        if SY:
            for r in range(16):
                c_prep_s(r)
            for r in range(8):
                c_prep_tail(r)
        else:
            c_prep(0, D // 16)
    wv_t()
    scan(7, bur, bui)
    for c in g3:
        c.wait()
    loop(0, NB, UA, a1)
    kv_final()
    loop(0, NB, UC, ya_block)
    for i in range(NB):
        out_cp(i, 0).wait()
        out_cp(i, 1).wait()


@jax.jit
def pallas_concat_heads__linear_kernel_hedgehog__ssm_conv_s5__prompt_kernel(A_x, A_wqkv, A_w_phi, A_wo, B_x, B_Lambda_re, B_Lambda_im, B_B_re, B_B_im,
              B_C_re, B_C_im, B_log_dt, B_Dskip):
    xa = A_x.reshape(S, D)
    xb = B_x.reshape(S, D)
    hbm = pl.BlockSpec(memory_space=pltpu.HBM)
    V = pltpu.VMEM
    out = pl.pallas_call(
        _kernel,
        in_specs=[hbm] * 13,
        out_specs=hbm,
        out_shape=jax.ShapeDtypeStruct((S, 2 * D), f32),
        scratch_shapes=[
            V((S, D), bf16), V((D, 3 * D), bf16), V((DH, DH, H), bf16), V((D, D), bf16), V((S, D), bf16),
            V((D,), bf16), V((D,), bf16), V((D, D), bf16), V((D, D), bf16), V((D, D), bf16), V((D, D), bf16),
            V((D,), bf16), V((D,), bf16),
            V((S, 2 * D), f32),
            V((D, 128), f32),
            V((3 * D // 2, D), u32),
            V((3 * NG, 7, MH // 2, 256), u32), V((3 * NG, MH, 128), u32), V((8, 64, 256), u32),
            V((NB, D, TB), u32),
            V((NPAIR, 48, 80), f32), V((NPAIR, 48, 80), bf16),
            V((D // 2, 2 * D), u32), V((7, 128, D), u32), V((D // 2, D), u32),
            V((12, 8, D), f32), V((2, 8, D), f32), V((8, 128), u32),
            V((NB, NL, NCH * WS, 128), u32), V((2, TB, D), f32), V((NB, 2 * NL, NCH * WS, 128), u32),
            V((416, 128), u32), pltpu.SemaphoreType.DMA((15,)), pltpu.SemaphoreType.DMA((2 * NB,)),
        ],
        compiler_params=pltpu.CompilerParams(vmem_limit_bytes=100 * 1024 * 1024),
    )(xa, A_wqkv, A_w_phi.transpose(1, 2, 0), A_wo, xb, B_Lambda_re, B_Lambda_im, B_B_re, B_B_im,
      B_C_re, B_C_im, B_log_dt, B_Dskip)
    return out.reshape(1, S, 2 * D)
```

```python
import math

import jax
import jax.numpy as jnp
import jax.experimental.pallas as pl
import jax.experimental.pallas.tpu as pltpu

S, D, H, DH = 2048, 640, 32, 20
TB = 256
NB = S // TB
NCH = 8
C = TB // NCH
WS = C // 2 + 4
NL = D // 128
NPAIR = H // 2
UNROLL = 2
LOG2E = 1.4426950408889634
BANDS = ((0, 160), (112, 288), (240, 400), (352, 528), (480, 640))
PORD = (0, 1, 5, 6, 4, 3, 2)

f32, bf16, u32 = jnp.float32, jnp.bfloat16, jnp.uint32
NN = (((1,), (0,)), ((), ()))
NT = (((1,), (1,)), ((), ()))
TN = (((0,), (0,)), ((), ()))


def _dot(a, b, dims):
    return jax.lax.dot_general(a, b, dims, preferred_element_type=f32)


def _w(x):
    return pltpu.bitcast(x.astype(bf16), u32)


def _b(x):
    return pltpu.bitcast(x, bf16)


def _cat0(xs):
    return jnp.concatenate(list(xs), axis=0)


def _cat1(xs):
    return jnp.concatenate(list(xs), axis=1)


def _lt(l):
    return slice(128 * l, 128 * (l + 1))


def _cmul(ar, ai, br, bi):
    return ar * br - ai * bi, ar * bi + ai * br


def _recip(x):
    r = pl.reciprocal(x, approx=True)
    return r * (2.0 - x * r)


def _par_red(op, rows):
    m = rows[0]
    for r in rows[1:]:
        m = op(m, r)
    m = op(m, pltpu.roll(m, 4, 0))
    return op(m, pltpu.roll(m, 2, 0))


def _phi_pair(p):
    rows = [p[8 * i:8 * i + 8] for i in range(5)]
    mx = _par_red(jnp.maximum, rows)
    mn = _par_red(jnp.minimum, rows)
    ep = [jnp.exp2(r - mx) for r in rows]
    en = [jnp.exp2(mn - r) for r in rows]
    rp = _recip(_par_red(jnp.add, ep))
    rn = _recip(_par_red(jnp.add, en))
    return _cat0([e * rp for e in ep] + [e * rn for e in en]).astype(bf16)


def _kernel(xa_h, wqkv_h, wphi_h, wo_h, xb_h, lre_h, lim_h, bre_h, bim_h, cre_h, cim_h, ldt_h, dsk_h,
            out_h,
            xa_v, wqkv_v, wphi_v, wo_v, xb_v, lre_v, lim_v, bre_v, bim_v, cre_v, cim_v, ldt_v, dsk_v,
            out_v,
            wp_ref, fg_ref, wt_ref, phiq_ref, kv_ref, kvl_ref, c2_ref, ct_ref, wo_ref,
            tab_ref, carry_ref, zero_ref, xs_ref, z_ref, bu_ref, hs_ref,
            sem_in, sem_out):

    def cp(src, dst, k):
        return pltpu.make_async_copy(src, dst, sem_in.at[k])

    def xb_cp(lo, hi, k):
        r = pl.ds(TB * lo, TB * (hi - lo))
        return cp(xb_h.at[r], xb_v.at[r], k)

    g0 = [cp(lre_h, lre_v, 0), cp(lim_h, lim_v, 1), cp(ldt_h, ldt_v, 2), cp(wphi_h, wphi_v, 3)]
    g1 = [cp(bre_h, bre_v, 4), xb_cp(0, 1, 5)]
    g2 = [cp(bim_h, bim_v, 6)]
    g3 = [xb_cp(1, 4, 7)]
    g4 = [xb_cp(4, NB, 8), cp(wqkv_h, wqkv_v, 9)]
    g5 = [cp(xa_h, xa_v, 10), cp(wo_h, wo_v, 11), cp(dsk_h, dsk_v, 12),
          cp(cre_h, cre_v, 13), cp(cim_h, cim_v, 14)]

    def start(g):
        for c in g:
            c.start()

    def wait(g):
        for c in g:
            c.wait()

    def rows_of(i):
        return pl.ds(pl.multiple_of(TB * i, TB), TB)

    def out_cp(i, part):
        c = pl.ds(D * part, D)
        return pltpu.make_async_copy(out_v.at[rows_of(i), c], out_h.at[rows_of(i), c],
                                     sem_out.at[2 * i + part])

    def lam_prep():
        lre = lre_v[...].astype(f32).reshape(1, D)
        lim = lim_v[...].astype(f32).reshape(1, D)
        dt = jnp.exp(ldt_v[...].astype(f32).reshape(1, D)).astype(bf16).astype(f32)
        mag = jnp.exp(dt * lre)
        ar = mag * jnp.cos(dt * lim)
        ai = mag * jnp.sin(dt * lim)
        nr, ni = ar - 1.0, ai
        den = lre * lre + lim * lim
        tab_ref[10] = jnp.broadcast_to(2.0 * (nr * lre + ni * lim) / den, (8, D))
        tab_ref[11] = jnp.broadcast_to(2.0 * (ni * lre - nr * lim) / den, (8, D))
        pr = jnp.broadcast_to(ar, (8, D))
        pi = jnp.broadcast_to(ai, (8, D))
        tab_ref[0] = pr
        tab_ref[1] = pi
        for _ in range(int(math.log2(C))):
            pr, pi = _cmul(pr, pi, pr, pi)
        sub = jax.lax.broadcasted_iota(jnp.int32, (8, D), 0)
        tr, ti = pr, pi
        for n, k in enumerate((1, 2, 4)):
            tab_ref[2 + 2 * n] = pr
            tab_ref[3 + 2 * n] = pi
            mr, mi = _cmul(tr, ti, pltpu.roll(tr, k, 0), pltpu.roll(ti, k, 0))
            tr = jnp.where(sub >= k, mr, tr)
            ti = jnp.where(sub >= k, mi, ti)
            pr, pi = _cmul(pr, pi, pr, pi)
        tab_ref[8] = tr
        tab_ref[9] = ti
        carry_ref[...] = jnp.zeros(carry_ref.shape, f32)
        zz = jnp.broadcast_to(lim[:, 0:128], (8, 128))
        zero_ref[...] = pltpu.bitcast(zz - zz, u32)

    def c_tile(r0, l, tok):
        cr2 = pltpu.bitcast(pltpu.bitcast(tab_ref[10, :, _lt(l)], u32) | tok, f32)
        cr2 = _cat0([cr2] * 2)
        ci2 = _cat0([tab_ref[11, :, _lt(l)]] * 2)
        rows = pl.ds(pl.multiple_of(r0, 16), 16)
        a = cre_v[rows, _lt(l)].astype(f32)
        b = cim_v[rows, _lt(l)].astype(f32)
        return a * cr2 - b * ci2, -(a * ci2 + b * cr2)

    def side_work(i):
        def strassen(r, l):
            def f(tok):
                b11, b21 = c_tile(16 * r, l, tok)
                b12, b22 = c_tile(256 + 16 * r, l, tok)
                t1 = b12 - b11
                t2 = b22 - t1
                for n, t in enumerate((b11, b21, b22, t2 - b21, t1, t2, b22 - b12)):
                    ct_ref[n, pl.ds(pl.multiple_of(8 * r, 8), 8), _lt(l)] = _w(t)
            return f

        def plain(ls):
            def f(tok):
                wr = pl.ds(pl.multiple_of(8 * i, 8), 8)
                for l in ls:
                    cr, ci = c_tile(512 + 16 * i, l, tok)
                    c2_ref[wr, _lt(l)] = _w(cr)
                    c2_ref[wr, _lt(NL + l)] = _w(ci)
                    wo_ref[pl.ds(pl.multiple_of(40 * i, 8), 40), _lt(l)] = (
                        pltpu.bitcast(wo_v[pl.ds(pl.multiple_of(80 * i, 16), 80), _lt(l)], u32)
                        | _cat0([tok] * 5))
            return f

        return ([strassen(2 * i + k, l) for k in range(2) for l in range(NL)]
                + [plain((0, 1, 2)), plain((3, 4))])

    def fold_lhs():
        for d in range(DH):
            t = wphi_v[d].astype(f32).T
            wp_ref[pl.ds(d, H, stride=DH), :] = _cat1([t, jnp.zeros((H, 128 - DH), f32)])
        sub = jax.lax.broadcasted_iota(jnp.int32, (8, 128), 0)
        lane = jax.lax.broadcasted_iota(jnp.int32, (8, 128), 1)
        selv = [(4 * v + (sub >> 1) == lane).astype(f32) for v in range(5)]
        off = 0
        for j, (lo, hi) in enumerate(BANDS):
            vs = range(lo // 8, hi // 8)
            sel = _cat0(selv[v % 5] for v in vs).astype(bf16)
            full = _dot(sel, wp_ref[_lt(j), :].astype(bf16), NT)
            key = (128 * j + lane) // DH - (sub & 1)
            fg_ref[off:off + (hi - lo) // 2, :] = _w(_cat0(
                jnp.where(key == 2 * (v // 5), full[8 * k:8 * k + 8], 0.0) for k, v in enumerate(vs)))
            off += (hi - lo) // 2

    def fold(part):
        for nt in range(NL):
            ps, off = [], 0
            for j, (lo, hi) in enumerate(BANDS):
                n = (hi - lo) // 2
                ps.append(_dot(_b(fg_ref[off:off + n, :]), wqkv_v[_lt(nt), _lt(NL * part + j)], NT) * LOG2E)
                off += n
            wt_ref[part * D // 2:(part + 1) * D // 2, _lt(nt)] = _w(_cat0(
                [ps[0][0:112], ps[0][112:160] + ps[1][0:48], ps[1][48:128], ps[1][128:176] + ps[2][0:48],
                 ps[2][48:112], ps[2][112:160] + ps[3][0:48], ps[3][48:128], ps[3][128:176] + ps[4][0:48],
                 ps[4][48:160]]))

    def wv_t():
        for nt in range(NL):
            wt_ref[D:3 * D // 2, _lt(nt)] = _w(wqkv_v[_lt(nt), 2 * D:3 * D].T.astype(f32))
        kv_ref[...] = jnp.zeros(kv_ref.shape, f32)

    def bu_mm(i, dep=None, mid=None):
        for l in range(NL):
            for j in range(NCH):
                xs_ref[i, l, pl.ds(WS * j, C // 2), :] = pltpu.bitcast(
                    xb_v[TB * i + C * j:TB * i + C * (j + 1), _lt(l)], u32)
        cols = []
        for l in range(NL):
            rows = []
            for c in range(C // 2):
                v = xs_ref[i, l, pl.ds(c, 8, stride=WS), :]
                rows.append(_cat0(
                    pltpu.unpack_elementwise(v, index=k, packed_dtype=bf16, unpacked_dtype=f32)
                    for k in range(2)).astype(bf16))
            cols.append(_cat0(rows))
        z = _cat1(cols)
        bur = _dot(z, bre_v[...], NT)
        if mid is not None:
            z_ref[...] = pltpu.bitcast(z, u32)
            bu_ref[0] = bur
            mid()
            z = _b(z_ref[...])
        if dep is not None:
            z0 = _b(pltpu.bitcast(z[0:16, 0:128], u32) | dep)
            z = _cat0([_cat1([z0, z[0:16, 128:]]), z[16:]])
        return bur, _dot(z, bim_v[...], NT)

    def scan(i, bur, bui):
        ar, ai = tab_ref[0], tab_ref[1]

        def step(hr, hi, c):
            mr, mi = _cmul(ar, ai, hr, hi)
            return mr + bur[8 * c:8 * c + 8], mi + bui[8 * c:8 * c + 8]

        hr, hi = bur[0:8], bui[0:8]
        for c in range(1, C):
            hr, hi = step(hr, hi, c)
        sub = jax.lax.broadcasted_iota(jnp.int32, (8, D), 0)
        for n, k in enumerate((1, 2, 4)):
            sr = jnp.where(sub >= k, pltpu.roll(hr, k, 0), 0.0)
            si = jnp.where(sub >= k, pltpu.roll(hi, k, 0), 0.0)
            mr, mi = _cmul(tab_ref[2 + 2 * n], tab_ref[3 + 2 * n], sr, si)
            hr, hi = hr + mr, hi + mi
        cr, ci = carry_ref[0], carry_ref[1]
        mr, mi = _cmul(tab_ref[8], tab_ref[9], cr, ci)
        gr, gi = hr + mr, hi + mi
        carry_ref[0] = jnp.broadcast_to(gr[7:8], (8, D))
        carry_ref[1] = jnp.broadcast_to(gi[7:8], (8, D))
        hr = jnp.where(sub == 0, cr, pltpu.roll(gr, 1, 0))
        hi = jnp.where(sub == 0, ci, pltpu.roll(gi, 1, 0))
        for c in range(0, C, 2):
            h0r, h0i = step(hr, hi, c)
            hr, hi = step(h0r, h0i, c + 1)
            pr = pltpu.pack_elementwise([h0r, hr], packed_dtype=bf16)
            pi = pltpu.pack_elementwise([h0i, hi], packed_dtype=bf16)
            for l in range(NL):
                hs_ref[i, l, pl.ds(c // 2, 8, stride=WS), :] = pr[:, _lt(l)]
                hs_ref[i, NL + l, pl.ds(c // 2, 8, stride=WS), :] = pi[:, _lt(l)]
        tok = pr[:, _lt(0)]
        for l in range(1, NL):
            tok = tok | pr[:, _lt(l)]
        return tok & zero_ref[...]

    def y_mm(i):
        a = [[_cat1(_b(_cat0(hs_ref[i, NL * k + l, pl.ds(WS * j, C // 2), :]
                             for j in range(4 * m, 4 * m + 4))) for l in range(NL))
              for k in range(2)] for m in range(2)]
        a11, a12, a21, a22 = (a[m][k].astype(f32) for m in range(2) for k in range(2))
        s1 = a21 + a22
        s2 = s1 - a11
        sa = (a[0][0], a[0][1], (a12 - s2).astype(bf16), a[1][1], s1.astype(bf16), s2.astype(bf16),
              (a11 - a21).astype(bf16))
        p = [None] * 7
        for n in PORD:
            p[n] = _dot(sa[n], _b(ct_ref[n]), NT)
        e = _dot(_cat0(_cat1(a[m]) for m in range(2)), _b(c2_ref[...]), NT)
        u2 = p[0] + p[5]
        u3 = u2 + p[6]
        y = _cat0([_cat1([p[0] + p[1], u2 + p[4] + p[2], e[0:128]]),
                   _cat1([u3 - p[3], u3 + p[4], e[128:]])])
        skip = (xb_v[rows_of(i), :] * dsk_v[...].reshape(1, D)).astype(f32)
        out_v[rows_of(i), D:2 * D] = y + skip
        out_cp(i, 1).start()

    def attn_kv(i):
        xa = xa_v[rows_of(i), :]
        ones = jnp.ones((8, TB), f32)
        pieces = side_work(i)
        for g in range(4):
            vt, pk, pq = [
                _dot(_b(wt_ref[part * D // 2 + 80 * g:part * D // 2 + 80 * (g + 1), :]), xa, NT)
                for part in (2, 1, 0)]
            for r in (vt, pk, pq):
                pieces.pop(0)(pltpu.bitcast(r[0:8, 0:128], u32) & zero_ref[...])
            for q in range(4):
                phik = _phi_pair(pk[40 * q:40 * q + 40])
                lhs = _cat0([vt[40 * q:40 * q + 40], ones]).astype(bf16)
                kv_ref[4 * g + q] += _dot(lhs, phik, NT)
            for q in range(4):
                p = 4 * g + q
                phiq_ref[i, 40 * p:40 * p + 40, :] = _w(_phi_pair(pq[40 * q:40 * q + 40]))

    def kv_final():
        m = jax.lax.broadcasted_iota(jnp.int32, (48, 80), 0)
        n = jax.lax.broadcasted_iota(jnp.int32, (48, 80), 1)
        msk = jnp.where(m < 40, m // 20, (m - 40) // 4) == n % 2
        for p in range(NPAIR):
            kvl_ref[p] = jnp.where(msk, kv_ref[p], 0.0).astype(bf16)

    def outputs(i):
        sub = jax.lax.broadcasted_iota(jnp.int32, (8, TB), 0)
        parts = []
        for p in range(NPAIR):
            res = _dot(kvl_ref[p], _b(phiq_ref[i, 40 * p:40 * p + 40, :]), NN)
            r = _recip(res[40:48] + 1e-6)
            rr = pltpu.roll(r, 4, 0)
            ra = jnp.where(sub < 4, r, rr)
            rc = jnp.where(sub >= 4, r, rr)
            parts += [res[0:8] * ra, res[8:16] * ra, res[16:24] * r, res[24:32] * rc, res[32:40] * rc]
        ot = _cat0(parts).astype(bf16)
        y_mm(i)
        out_v[rows_of(i), 0:D] = _dot(ot, _b(wo_ref[...]), TN)
        out_cp(i, 0).start()

    def loop(fn):
        def body(k, carry):
            for j in range(UNROLL):
                fn(UNROLL * k + j)
            return carry
        jax.lax.fori_loop(0, NB // UNROLL, body, 0)

    start(g0 + g1)
    wait(g0)
    lam_prep()
    start(g2)
    fold_lhs()
    wait(g1)
    start(g3)
    _, bui = bu_mm(0, mid=lambda: wait(g2))
    bu_ref[1] = bui
    wait(g3)
    start(g4)
    tok = scan(0, bu_ref[0], bu_ref[1])
    scan(1, *bu_mm(1, tok))
    scan(2, *bu_mm(2))
    bu_ref[0], bu_ref[1] = bu_mm(3)
    wait(g4)
    start(g5)
    tok = scan(3, bu_ref[0], bu_ref[1])
    scan(4, *bu_mm(4, tok))
    scan(5, *bu_mm(5))
    bu = bu_mm(6)
    fold(0)
    scan(6, *bu)
    bu = bu_mm(7)
    fold(1)
    wv_t()
    scan(7, *bu)
    wait(g5)
    loop(attn_kv)
    kv_final()
    loop(outputs)
    for i in range(NB):
        out_cp(i, 0).wait()
        out_cp(i, 1).wait()


@jax.jit
def pallas_concat_heads__linear_kernel_hedgehog__ssm_conv_s5__prompt_kernel(
    A_x: jax.Array,
    A_wqkv: jax.Array,
    A_w_phi: jax.Array,
    A_wo: jax.Array,
    B_x: jax.Array,
    B_Lambda_re: jax.Array,
    B_Lambda_im: jax.Array,
    B_B_re: jax.Array,
    B_B_im: jax.Array,
    B_C_re: jax.Array,
    B_C_im: jax.Array,
    B_log_dt: jax.Array,
    B_Dskip: jax.Array,
):
    hbm = pl.BlockSpec(memory_space=pltpu.HBM)
    V = pltpu.VMEM
    out = pl.pallas_call(
        _kernel,
        in_specs=[hbm] * 13,
        out_specs=hbm,
        out_shape=jax.ShapeDtypeStruct((S, 2 * D), f32),
        scratch_shapes=[
            V((S, D), bf16), V((D, 3 * D), bf16), V((DH, DH, H), bf16), V((D, D), bf16), V((S, D), bf16),
            V((D,), bf16), V((D,), bf16), V((D, D), bf16), V((D, D), bf16), V((D, D), bf16), V((D, D), bf16),
            V((D,), bf16), V((D,), bf16),
            V((S, 2 * D), f32),
            V((D, 128), f32), V((416, 128), u32), V((3 * D // 2, D), u32), V((NB, D, TB), u32),
            V((NPAIR, 48, 80), f32), V((NPAIR, 48, 80), bf16),
            V((64, 2 * D), u32), V((7, 128, D), u32), V((D // 2, D), u32),
            V((12, 8, D), f32), V((2, 8, D), f32), V((8, 128), u32),
            V((NB, NL, NCH * WS, 128), u32), V((TB // 2, D), u32), V((2, TB, D), f32),
            V((NB, 2 * NL, NCH * WS, 128), u32),
            pltpu.SemaphoreType.DMA((15,)), pltpu.SemaphoreType.DMA((2 * NB,)),
        ],
        compiler_params=pltpu.CompilerParams(vmem_limit_bytes=100 * 1024 * 1024),
    )(A_x.reshape(S, D), A_wqkv, A_w_phi.transpose(1, 2, 0), A_wo, B_x.reshape(S, D), B_Lambda_re,
      B_Lambda_im, B_B_re, B_B_im, B_C_re, B_C_im, B_log_dt, B_Dskip)
    return out.reshape(1, S, 2 * D)
```
